```python
import os as _os
_os.environ.setdefault("JAX_PLATFORMS", "cpu")
import jax
import jax.numpy as jnp

def _softmax(x, axis=-1):
    return jax.nn.softmax(x, axis=axis)
def _gelu(x):
    return jax.nn.gelu(x, approximate=True)
def _silu(x):
    return jax.nn.silu(x)
def _sigmoid(x):
    return jax.nn.sigmoid(x)
def _layernorm(x, axis=-1, eps=1e-5):
    m = jnp.mean(x, axis=axis, keepdims=True)
    v = jnp.var(x, axis=axis, keepdims=True)
    return (x - m) / jnp.sqrt(v + eps)
def _scatter_add(tgt, idx, src, axis=0):
    return tgt.at[idx].add(src)
def _segment_sum(src, seg, n):
    return jax.ops.segment_sum(src, seg, n)
class _Rng:
    def __init__(self, key):
        self._k = key
    def _next(self):
        self._k, sub = jax.random.split(self._k)
        return sub
    def normal(self, shape):
        return jax.random.normal(self._next(), shape, dtype=jnp.bfloat16)
    def randint(self, lo, hi, shape):
        return jax.random.randint(self._next(), shape, lo, hi, dtype=jnp.int32)
    def uniform(self, shape, lo=0.0, hi=1.0):
        return jax.random.uniform(self._next(), shape, jnp.bfloat16, lo, hi)
    def permutation(self, n):
        return jax.random.permutation(self._next(), n)


kernel_name = 'concat_heads__sliding_local_dilated__sliding_block__prompt'

def setup_inputs():
    _rng = _Rng(jax.random.key(int.from_bytes(__import__("os").urandom(4), "little")))
    _w = (lambda a: (lambda t: t.astype(jnp.bfloat16) if jnp.issubdtype(t.dtype, jnp.floating) else t)(jnp.asarray(a)))
    def _A_setup():
        B, S, D = 1, 2048, 1024
        return {
            "x": _w((lambda *s: _rng.normal(s) * 0.2)(B, S, D)),
            "wqkv": _w((lambda *s: _rng.normal(s) * 0.2)(D, 3 * D)),
            "wo": _w((lambda *s: _rng.normal(s) * 0.05)(D, D)),
        }
    _A_in = _A_setup()

    def _B_setup():
        B, S, D = 1, 2048, 1024
        return {
            "x": _w((lambda *s: _rng.normal(s) * 0.2)(B, S, D)),
            "wqkv": _w((lambda *s: _rng.normal(s) * 0.2)(D, 3 * D)),
            "wo": _w((lambda *s: _rng.normal(s) * 0.05)(D, D)),
        }
    _B_in = _B_setup()

    return {
        "A_x": _A_in["x"],
        "A_wqkv": _A_in["wqkv"],
        "A_wo": _A_in["wo"],
        "B_x": _B_in["x"],
        "B_wqkv": _B_in["wqkv"],
        "B_wo": _B_in["wo"],
    }

def reference(A_x, A_wqkv, A_wo, B_x, B_wqkv, B_wo):
    def _A_ref(x, wqkv, wo):
        B, S, D = x.shape
        H = 32; Dh = D // H
        W, dil = 8, 2
        qkv = (lambda x, *d: x.transpose(*d))((x @ wqkv).reshape(B, S, 3, H, Dh), 2, 0, 3, 1, 4)
        q, k, v = qkv[0], qkv[1], qkv[2]
        scale = Dh ** -0.5
        pos = jnp.arange(S)
        off = jnp.arange(W) * dil
        idx = pos[:, None] - off[None, :]
        mask = idx >= 0
        idx_c = jnp.where(mask, idx, 0).reshape(-1)
        kg = k[:, :, idx_c, :].reshape(B, H, S, W, Dh)
        vg = v[:, :, idx_c, :].reshape(B, H, S, W, Dh)
        logits = jnp.einsum("bhsd,bhswd->bhsw", q, kg) * scale
        logits = jnp.where(mask[None, None, :, :], logits, -1e9)
        attn = _softmax(logits, axis=-1)
        o = jnp.einsum("bhsw,bhswd->bhsd", attn, vg)
        return (lambda x, *d: x.transpose(*d))(o, 0, 2, 1, 3).reshape(B, S, D) @ wo

    def _B_ref(x, wqkv, wo):
        B, S, D = x.shape
        H = 32; Dh = D // H; W = 256
        qkv = (lambda x, *d: x.transpose(*d))((x @ wqkv).reshape(B, S, 3, H, Dh), 2, 0, 3, 1, 4)
        q, k, v = qkv[0], qkv[1], qkv[2]
        scores = jnp.einsum("bhqd,bhkd->bhqk", q, k) * (Dh ** -0.5)
        idx = jnp.arange(S)
        mask = (idx[:, None] - idx[None, :] >= 0) & (idx[:, None] - idx[None, :] < W)
        scores = jnp.where(mask[None, None], scores, -1e9)
        p = _softmax(scores, axis=-1)
        o = jnp.einsum("bhqk,bhkd->bhqd", p, v)
        return (lambda x, *d: x.transpose(*d))(o, 0, 2, 1, 3).reshape(B, S, D) @ wo

    a = _A_ref(A_x, A_wqkv, A_wo)
    b = _B_ref(B_x, B_wqkv, B_wo)
    return jnp.concatenate([a, b], axis=-1)
```

```python
import functools

import jax
import jax.numpy as jnp
import jax.experimental.pallas as pl
import jax.experimental.pallas.tpu as pltpu

S = 2048
D = 1024
H = 32
DH = 32
TM = 256
PAD = 256
NG = D // 128
NEG = -1e9
SCALE = DH ** -0.5


def _stack_masked_q(qg, rows):
    lane = jax.lax.broadcasted_iota(jnp.int32, (rows, 128), 1)
    parts = [jnp.where((lane // DH) == j, qg, jnp.zeros_like(qg)) for j in range(4)]
    return jnp.concatenate(parts, axis=0)


def _select_heads(o, rows):
    lane = jax.lax.broadcasted_iota(jnp.int32, (rows, 128), 1)
    hid = lane // DH
    res = o[0:rows]
    for j in range(1, 4):
        res = jnp.where(hid == j, o[j * rows:(j + 1) * rows], res)
    return res


def _attn_b(q_scr, k_scr, v_scr, o_scr, row0):
    QB = 128
    r = jax.lax.broadcasted_iota(jnp.int32, (4 * QB, QB), 0) % QB
    c = jax.lax.broadcasted_iota(jnp.int32, (4 * QB, QB), 1)
    tri = r >= c
    for qb in range(TM // QB):
        g0 = row0 + qb * QB
        kstart = pl.multiple_of(g0, QB)
        has_m1 = g0 >= QB
        has_m2 = g0 >= 2 * QB
        for g in range(NG):
            lanes = slice(g * 128, (g + 1) * 128)
            qs = _stack_masked_q(q_scr[qb * QB:(qb + 1) * QB, lanes], QB)
            kg = k_scr[pl.ds(kstart, 3 * QB), lanes]
            vg = v_scr[pl.ds(kstart, 3 * QB), lanes]
            s = jax.lax.dot_general(qs, kg, (((1,), (1,)), ((), ())),
                                    preferred_element_type=jnp.float32)
            s0 = jnp.where(has_m2, s[:, 0:QB], NEG)
            s1 = jnp.where(has_m1, s[:, QB:2 * QB], NEG)
            s2 = s[:, 2 * QB:3 * QB]
            comb = jnp.where(tri, s2, s0)
            m = jnp.max(jnp.maximum(comb, s1), axis=-1, keepdims=True)
            p1 = jnp.exp(s1 - m)
            pc = jnp.exp(comb - m)
            l = jnp.sum(p1 + pc, axis=-1, keepdims=True)
            zero = jnp.zeros_like(pc)
            p = jnp.concatenate([jnp.where(tri, zero, pc), p1, jnp.where(tri, pc, zero)],
                                axis=1).astype(jnp.bfloat16)
            o = jnp.dot(p, vg, preferred_element_type=jnp.float32)
            o = o / l
            o_scr[qb * QB:(qb + 1) * QB, lanes] = _select_heads(o, QB).astype(jnp.bfloat16)


def _attn_a(q_scr, k_scr, v_scr, o_scr, row0):
    QB = 64
    KB = QB + 16
    r = jax.lax.broadcasted_iota(jnp.int32, (4 * QB, KB), 0) % QB
    c = jax.lax.broadcasted_iota(jnp.int32, (4 * QB, KB), 1)
    delta = r + 16 - c
    band = (delta >= 0) & (delta <= 14) & ((delta % 2) == 0)
    for qb in range(TM // QB):
        g0 = row0 + qb * QB
        kstart = pl.multiple_of(g0 + (PAD - 16), 16)
        valid = band & ((c + (g0 - 16)) >= 0)
        for g in range(NG):
            lanes = slice(g * 128, (g + 1) * 128)
            qs = _stack_masked_q(q_scr[qb * QB:(qb + 1) * QB, lanes], QB)
            kg = k_scr[pl.ds(kstart, KB), lanes]
            vg = v_scr[pl.ds(kstart, KB), lanes]
            s = jax.lax.dot_general(qs, kg, (((1,), (1,)), ((), ())),
                                    preferred_element_type=jnp.float32)
            s = jnp.where(valid, s, NEG)
            m = jnp.max(s, axis=-1, keepdims=True)
            p = jnp.exp(s - m)
            p = jnp.where(valid, p, 0.0)
            l = jnp.sum(p, axis=-1, keepdims=True)
            o = jnp.dot(p.astype(jnp.bfloat16), vg, preferred_element_type=jnp.float32)
            o = o / l
            o_scr[qb * QB:(qb + 1) * QB, lanes] = _select_heads(o, QB).astype(jnp.bfloat16)


def _kernel(xa_ref, wqkva_ref, woa_ref, xb_ref, wqkvb_ref, wob_ref, out_ref,
            q_scr, k_scr, v_scr, o_scr):
    b = pl.program_id(0)
    i = pl.program_id(1)
    row0 = i * TM

    @pl.when(i == 0)
    def _():
        k_scr[0:PAD, :] = jnp.zeros((PAD, D), jnp.bfloat16)
        v_scr[0:PAD, :] = jnp.zeros((PAD, D), jnp.bfloat16)

    def branch(x_ref, wqkv_ref, wo_ref, attn):
        x = x_ref[...]
        dst = pl.multiple_of(row0 + PAD, TM)
        q = jnp.dot(x, wqkv_ref[:, 0:D], preferred_element_type=jnp.float32)
        q_scr[...] = (q.astype(jnp.bfloat16).astype(jnp.float32) * SCALE).astype(jnp.bfloat16)
        k = jnp.dot(x, wqkv_ref[:, D:2 * D], preferred_element_type=jnp.float32)
        k_scr[pl.ds(dst, TM), :] = k.astype(jnp.bfloat16)
        v = jnp.dot(x, wqkv_ref[:, 2 * D:3 * D], preferred_element_type=jnp.float32)
        v_scr[pl.ds(dst, TM), :] = v.astype(jnp.bfloat16)
        attn(q_scr, k_scr, v_scr, o_scr, row0)
        out_ref[...] = jnp.dot(o_scr[...], wo_ref[...],
                               preferred_element_type=jnp.float32).astype(out_ref.dtype)

    @pl.when(b == 0)
    def _():
        branch(xa_ref, wqkva_ref, woa_ref, _attn_a)

    @pl.when(b == 1)
    def _():
        branch(xb_ref, wqkvb_ref, wob_ref, _attn_b)


@jax.jit
def pallas_concat_heads__sliding_local_dilated__sliding_block__prompt_kernel(
    A_x: jax.Array,
    A_wqkv: jax.Array,
    A_wo: jax.Array,
    B_x: jax.Array,
    B_wqkv: jax.Array,
    B_wo: jax.Array,
):
    nb = S // TM
    xa = A_x.reshape(S, D)
    xb = B_x.reshape(S, D)
    full = lambda shape: pl.BlockSpec(shape, lambda b, i: (0, 0))
    out = pl.pallas_call(
        _kernel,
        grid=(2, nb),
        in_specs=[
            pl.BlockSpec((TM, D), lambda b, i: (i * (1 - b) + (nb - 1) * b, 0)),
            full((D, 3 * D)),
            full((D, D)),
            pl.BlockSpec((TM, D), lambda b, i: (i * b, 0)),
            full((D, 3 * D)),
            full((D, D)),
        ],
        out_specs=pl.BlockSpec((TM, D), lambda b, i: (i, b)),
        out_shape=jax.ShapeDtypeStruct((S, 2 * D), jnp.bfloat16),
        scratch_shapes=[
            pltpu.VMEM((TM, D), jnp.bfloat16),
            pltpu.VMEM((S + PAD, D), jnp.bfloat16),
            pltpu.VMEM((S + PAD, D), jnp.bfloat16),
            pltpu.VMEM((TM, D), jnp.bfloat16),
        ],
        compiler_params=pltpu.CompilerParams(
            dimension_semantics=("arbitrary", "arbitrary"),
            vmem_limit_bytes=100 * 1024 * 1024,
        ),
    )(xa, A_wqkv, A_wo, xb, B_wqkv, B_wo)
    return out.reshape(1, S, 2 * D)
```

```python
import jax
import jax.numpy as jnp
import jax.experimental.pallas as pl
import jax.experimental.pallas.tpu as pltpu

S = 2048
D = 1024
H = 32
DH = 32
TM = 256
PAD = 256
NG = D // 128
NEG = -1e9
SCALE = DH ** -0.5
LOG2E = 1.4426950408889634


def _stack_masked_q(qg, rows):
    lane = jax.lax.broadcasted_iota(jnp.int32, (rows, 128), 1)
    parts = [jnp.where((lane // DH) == j, qg, jnp.zeros_like(qg)) for j in range(4)]
    return jnp.concatenate(parts, axis=0)


def _select_heads(o, l, rows):
    lane = jax.lax.broadcasted_iota(jnp.int32, (rows, 128), 1)
    hid = lane // DH
    res = o[0:rows]
    den = jnp.broadcast_to(l[0:rows], (rows, 128))
    for j in range(1, 4):
        sel = hid == j
        res = jnp.where(sel, o[j * rows:(j + 1) * rows], res)
        den = jnp.where(sel, l[j * rows:(j + 1) * rows], den)
    return res / den


def _attn_b(qkv_scr, o_scr, row0):
    QB = 128
    r = jax.lax.broadcasted_iota(jnp.int32, (4 * QB, QB), 0) % QB
    c = jax.lax.broadcasted_iota(jnp.int32, (4 * QB, QB), 1)
    tri = r >= c
    for qb in range(TM // QB):
        g0 = row0 + qb * QB
        kstart = pl.multiple_of(g0, QB)
        qstart = pl.multiple_of(g0 + PAD, QB)
        has_m1 = g0 >= QB
        has_m2 = g0 >= 2 * QB
        for g in range(NG):
            lanes = slice(g * 128, (g + 1) * 128)
            klanes = slice(D + g * 128, D + (g + 1) * 128)
            vlanes = slice(2 * D + g * 128, 2 * D + (g + 1) * 128)
            qs = _stack_masked_q(qkv_scr[pl.ds(qstart, QB), lanes], QB)
            kg = qkv_scr[pl.ds(kstart, 3 * QB), klanes]
            vg = qkv_scr[pl.ds(kstart, 3 * QB), vlanes]
            s = jax.lax.dot_general(qs, kg, (((1,), (1,)), ((), ())),
                                    preferred_element_type=jnp.float32)
            s0 = jnp.where(has_m2, s[:, 0:QB], NEG)
            s1 = jnp.where(has_m1, s[:, QB:2 * QB], NEG)
            s2 = s[:, 2 * QB:3 * QB]
            comb = jnp.where(tri, s2, s0)
            m = jnp.max(jnp.maximum(comb, s1), axis=-1, keepdims=True)
            p1 = jnp.exp2(s1 - m)
            pc = jnp.exp2(comb - m)
            l = jnp.sum(p1 + pc, axis=-1, keepdims=True)
            zero = jnp.zeros_like(pc)
            p = jnp.concatenate([jnp.where(tri, zero, pc), p1, jnp.where(tri, pc, zero)],
                                axis=1).astype(jnp.bfloat16)
            o = jnp.dot(p, vg, preferred_element_type=jnp.float32)
            o_scr[qb * QB:(qb + 1) * QB, lanes] = _select_heads(o, l, QB).astype(jnp.bfloat16)
            yield


def _attn_a(qkv_scr, o_scr, row0):
    QB = 64
    KB = QB + 16
    r = jax.lax.broadcasted_iota(jnp.int32, (4 * QB, KB), 0) % QB
    c = jax.lax.broadcasted_iota(jnp.int32, (4 * QB, KB), 1)
    delta = r + 16 - c
    band = (delta >= 0) & (delta <= 14) & ((delta % 2) == 0)
    for qb in range(TM // QB):
        g0 = row0 + qb * QB
        kstart = pl.multiple_of(g0 + (PAD - 16), 16)
        qstart = pl.multiple_of(g0 + PAD, QB)
        valid = band & ((c + (g0 - 16)) >= 0)
        for g in range(NG):
            lanes = slice(g * 128, (g + 1) * 128)
            klanes = slice(D + g * 128, D + (g + 1) * 128)
            vlanes = slice(2 * D + g * 128, 2 * D + (g + 1) * 128)
            qs = _stack_masked_q(qkv_scr[pl.ds(qstart, QB), lanes], QB)
            kg = qkv_scr[pl.ds(kstart, KB), klanes]
            vg = qkv_scr[pl.ds(kstart, KB), vlanes]
            s = jax.lax.dot_general(qs, kg, (((1,), (1,)), ((), ())),
                                    preferred_element_type=jnp.float32)
            s = jnp.where(valid, s, NEG)
            m = jnp.max(s, axis=-1, keepdims=True)
            p = jnp.exp2(s - m)
            l = jnp.sum(p, axis=-1, keepdims=True)
            o = jnp.dot(p.astype(jnp.bfloat16), vg, preferred_element_type=jnp.float32)
            o_scr[qb * QB:(qb + 1) * QB, lanes] = _select_heads(o, l, QB).astype(jnp.bfloat16)
            yield


WO_AT = 4
NCH = 12
CW = 3 * D // NCH


def _kernel(xa_ref, wqkva_hbm, woa_hbm, xb_ref, wqkvb_hbm, wob_hbm, out_ref,
            qkva_scr, qkvb_scr, oa_scr, ob_scr, wqkva, woa, wqkvb, wob, sem_a, sem_b):
    i = pl.program_id(0)
    row0 = i * TM
    dst = pl.multiple_of(row0 + PAD, TM)

    def chunk_copy(src, dstw, sem, c):
        return pltpu.make_async_copy(src.at[:, pl.ds(c * CW, CW)],
                                     dstw.at[:, pl.ds(c * CW, CW)], sem.at[c])

    def wo_copies():
        return (pltpu.make_async_copy(woa_hbm, woa, sem_a.at[NCH]),
                pltpu.make_async_copy(wob_hbm, wob, sem_b.at[NCH]))

    def project(x_ref, wqkv_ref, qkv_scr):
        x = x_ref[...]
        q = jnp.dot(x, wqkv_ref[:, 0:D], preferred_element_type=jnp.float32)
        q = q.astype(jnp.bfloat16).astype(jnp.float32) * (SCALE * LOG2E)
        qkv_scr[pl.ds(dst, TM), 0:D] = q.astype(jnp.bfloat16)
        kv = jnp.dot(x, wqkv_ref[:, D:3 * D], preferred_element_type=jnp.float32)
        qkv_scr[pl.ds(dst, TM), D:3 * D] = kv.astype(jnp.bfloat16)

    @pl.when(i == 0)
    def _():
        for c in range(NCH):
            chunk_copy(wqkva_hbm, wqkva, sem_a, c).start()
        qkva_scr[0:PAD, :] = jnp.zeros((PAD, 3 * D), jnp.bfloat16)
        qkvb_scr[0:PAD, :] = jnp.zeros((PAD, 3 * D), jnp.bfloat16)

        def stream(x_ref, src, w, sem, qkv_scr, nxt):
            def body(c, carry):
                chunk_copy(src, w, sem, c).wait()
                nxt(c)
                col = pl.multiple_of(c * CW, CW)
                y = jnp.dot(x_ref[...], w[:, pl.ds(col, CW)],
                            preferred_element_type=jnp.float32)
                f = jnp.where(c < D // CW, SCALE * LOG2E, 1.0).astype(jnp.float32)
                y = y.astype(jnp.bfloat16).astype(jnp.float32) * f
                qkv_scr[pl.ds(dst, TM), pl.ds(col, CW)] = y.astype(jnp.bfloat16)
                return carry
            jax.lax.fori_loop(0, NCH, body, 0)

        def start_b(c):
            chunk_copy(wqkvb_hbm, wqkvb, sem_b, c).start()

        def start_wo(c):
            @pl.when(c == WO_AT)
            def _():
                for cp in wo_copies():
                    cp.start()

        stream(xa_ref, wqkva_hbm, wqkva, sem_a, qkva_scr, start_b)
        stream(xb_ref, wqkvb_hbm, wqkvb, sem_b, qkvb_scr, start_wo)
        for cp in wo_copies():
            cp.wait()

    @pl.when(i > 0)
    def _():
        project(xa_ref, wqkva, qkva_scr)
        project(xb_ref, wqkvb, qkvb_scr)

    ga = _attn_a(qkva_scr, oa_scr, row0)
    gb = _attn_b(qkvb_scr, ob_scr, row0)
    for _ in range(2 * NG):
        next(ga)
        next(ga)
        next(gb)
    out_ref[:, 0:D] = jnp.dot(oa_scr[...], woa[...],
                              preferred_element_type=jnp.float32).astype(out_ref.dtype)
    out_ref[:, D:2 * D] = jnp.dot(ob_scr[...], wob[...],
                                  preferred_element_type=jnp.float32).astype(out_ref.dtype)


@jax.jit
def pallas_concat_heads__sliding_local_dilated__sliding_block__prompt_kernel(
    A_x: jax.Array,
    A_wqkv: jax.Array,
    A_wo: jax.Array,
    B_x: jax.Array,
    B_wqkv: jax.Array,
    B_wo: jax.Array,
):
    nb = S // TM
    xa = A_x.reshape(S, D)
    xb = B_x.reshape(S, D)
    hbm = pl.BlockSpec(memory_space=pl.ANY)
    out = pl.pallas_call(
        _kernel,
        grid=(nb,),
        in_specs=[
            pl.BlockSpec((TM, D), lambda i: (i, 0)),
            hbm,
            hbm,
            pl.BlockSpec((TM, D), lambda i: (i, 0)),
            hbm,
            hbm,
        ],
        out_specs=pl.BlockSpec((TM, 2 * D), lambda i: (i, 0)),
        out_shape=jax.ShapeDtypeStruct((S, 2 * D), jnp.bfloat16),
        scratch_shapes=[
            pltpu.VMEM((S + PAD, 3 * D), jnp.bfloat16),
            pltpu.VMEM((S + PAD, 3 * D), jnp.bfloat16),
            pltpu.VMEM((TM, D), jnp.bfloat16),
            pltpu.VMEM((TM, D), jnp.bfloat16),
            pltpu.VMEM((D, 3 * D), jnp.bfloat16),
            pltpu.VMEM((D, D), jnp.bfloat16),
            pltpu.VMEM((D, 3 * D), jnp.bfloat16),
            pltpu.VMEM((D, D), jnp.bfloat16),
            pltpu.SemaphoreType.DMA((NCH + 1,)),
            pltpu.SemaphoreType.DMA((NCH + 1,)),
        ],
        compiler_params=pltpu.CompilerParams(
            dimension_semantics=("arbitrary",),
            vmem_limit_bytes=110 * 1024 * 1024,
        ),
    )(xa, A_wqkv, A_wo, xb, B_wqkv, B_wo)
    return out.reshape(1, S, 2 * D)
```
